```python
import jax
import jax.numpy as jnp

def _softmax(x, axis=-1):
    return jax.nn.softmax(x, axis=axis)
def _gelu(x):
    return jax.nn.gelu(x, approximate=True)
def _silu(x):
    return jax.nn.silu(x)
def _sigmoid(x):
    return jax.nn.sigmoid(x)
def _layernorm(x, axis=-1, eps=1e-5):
    m = jnp.mean(x, axis=axis, keepdims=True)
    v = jnp.var(x, axis=axis, keepdims=True)
    return (x - m) / jnp.sqrt(v + eps)
def _scatter_add(tgt, idx, src, axis=0):
    return tgt.at[idx].add(src)
def _segment_sum(src, seg, n):
    return jax.ops.segment_sum(src, seg, n)
class _Rng:
    def __init__(self, key):
        self._k = key
    def _next(self):
        self._k, sub = jax.random.split(self._k)
        return sub
    def normal(self, shape):
        return jax.random.normal(self._next(), shape, dtype=jnp.bfloat16)
    def randint(self, lo, hi, shape):
        return jax.random.randint(self._next(), shape, lo, hi, dtype=jnp.int32)
    def uniform(self, shape, lo=0.0, hi=1.0):
        return jax.random.uniform(self._next(), shape, jnp.bfloat16, lo, hi)
    def permutation(self, n):
        return jax.random.permutation(self._next(), n)


kernel_name = 'sequential_preLN__spectral_gfnet__glu_gated_bilinear__prompt'

def _fwd_setup_inputs():
    _rng = _Rng(jax.random.key(int.from_bytes(__import__("os").urandom(4), "little")))
    _w = (lambda a: (lambda t: t.astype(jnp.bfloat16) if jnp.issubdtype(t.dtype, jnp.floating) else t)(jnp.asarray(a)))
    def _A_setup():
        B, S, D = 1, 2048, 512
        Df = D // 2 + 1
        return {
            "x": _w((lambda *s: _rng.normal(s) * 0.05)(B, S, D)),
            "w_r": _w((lambda *s: _rng.normal(s) * 0.05)(S, Df) * 0.02),
            "w_i": _w((lambda *s: _rng.normal(s) * 0.05)(S, Df) * 0.02),
        }
    _A_in = _A_setup()

    def _B_setup():
        B, S, D, F = 1, 2048, 512, 1376
        return {
            "x": _w((lambda *s: _rng.normal(s) * 0.05)(B, S, D)),
            "w_gate": _w((lambda *s: _rng.normal(s) * 0.05)(D, F) * (D ** -0.5)),
            "w_up": _w((lambda *s: _rng.normal(s) * 0.05)(D, F) * (D ** -0.5)),
            "w_down": _w((lambda *s: _rng.normal(s) * 0.05)(F, D) * (F ** -0.5)),
        }
    _B_in = _B_setup()

    return {
        "A_x": _A_in["x"],
        "A_w_r": _A_in["w_r"],
        "A_w_i": _A_in["w_i"],
        "B_x": _B_in["x"],
        "B_w_gate": _B_in["w_gate"],
        "B_w_up": _B_in["w_up"],
        "B_w_down": _B_in["w_down"],
    }

def _fwd_reference(A_x, A_w_r, A_w_i, B_x, B_w_gate, B_w_up, B_w_down):
    def _A_ref(x, w_r, w_i):
        B, S, D = x.shape
        X = (lambda x, axes=(-2,-1): jnp.fft.rfft2(x.astype(jnp.float32), axes=axes))(x, axes=(-2, -1))
        W = w_r + 1j * w_i
        X = X * W
        y = (lambda x, s, axes=(-2,-1): jnp.fft.irfft2(x, s=s, axes=axes).astype(jnp.bfloat16))(X, (S, D), axes=(-2, -1))
        return y

    def _B_ref(x, w_gate, w_up, w_down):
        g = jnp.einsum("bsd,df->bsf", x, w_gate)
        u = jnp.einsum("bsd,df->bsf", x, w_up)
        h = g * u
        return jnp.einsum("bsf,fd->bsd", h, w_down)

    x = A_x
    h = x + _A_ref(_layernorm(x, axis=-1), A_w_r, A_w_i)
    h2 = h + _B_ref(_layernorm(h, axis=-1), B_w_gate, B_w_up, B_w_down)
    return h2


def setup_inputs():
    _inp = _fwd_setup_inputs()
    _gk = jax.random.fold_in(jax.random.key(int.from_bytes(__import__("os").urandom(4), "little")), 2**31 - 1)
    _shapes = [[1, 2048, 512]]
    _dtypes = ['bfloat16']
    _gks = jax.random.split(_gk, len(_shapes))
    _gs = [jax.random.normal(k, s, dtype=jnp.dtype(d)) * 0.05 for k, s, d in zip(_gks, _shapes, _dtypes)]
    _inp["grad_out"] = _gs[0]
    return _inp

def reference(A_x, A_w_r, A_w_i, B_w_gate, B_w_up, B_w_down, B_x, grad_out):
    _const = dict(B_x=B_x)
    def _f(*_d):
        return _fwd_reference(**{'A_x': _d[0], 'A_w_r': _d[1], 'A_w_i': _d[2], 'B_w_gate': _d[3], 'B_w_up': _d[4], 'B_w_down': _d[5], **_const})
    _out, _vjp = jax.vjp(_f, A_x, A_w_r, A_w_i, B_w_gate, B_w_up, B_w_down)
    _grads = _vjp(grad_out)
    _out0 = jnp.asarray(_out)
    return (_out0, *[jnp.asarray(_g) for _g in _grads])
```

```python
import functools
import numpy as np
import jax
import jax.numpy as jnp
from jax.experimental import pallas as pl
from jax.experimental.pallas import tpu as pltpu

S, D, F = 2048, 512, 1376
NM = 257
NR = 272
EPS = 1e-5
TS = 256
NT = S // TS
f32 = jnp.float32
bf16 = jnp.bfloat16
P = functools.partial


def _consts():
    mo = np.concatenate([np.arange(64) * 4, np.arange(64) * 4 + 2, np.arange(128) * 2 + 1])
    d2 = np.arange(128)

    def cs(m):
        th = 2 * np.pi * np.outer(m, d2) / D
        return np.cos(th), np.sin(th)

    c0, s0 = cs(mo[:64]); c2, s2 = cs(mo[64:128]); co, so = cs(mo[128:256])
    FD0 = np.zeros((144, 128)); FD0[:64] = c0; FD0[64] = np.cos(np.pi * d2); FD0[80:144] = -s0
    FD2 = np.concatenate([c2, -s2], 0)
    sig = np.where(mo[128:256] % 4 == 1, 1.0, -1.0)[:, None]
    FDo = np.block([[co, -so + sig * co], [-sig * so - co, np.zeros((128, 128))]])
    sc = 2.0 / (S * D)
    ID0 = np.concatenate([c0 * sc, -s0 * sc], 0)
    ID0[0] = 1.0 / (S * D)
    ID0[64] = np.cos(np.pi * d2) / (S * D)
    ID2 = np.concatenate([c2 * sc, -s2 * sc], 0)
    IDo = np.block([[co * sc, -sig * so * sc], [-so * sc, -sig * co * sc]])
    a = np.arange(128)
    J2 = ((a[:, None] + a[None, :]) % 128 == 0).astype(np.float64)
    small = np.zeros((912, 256))
    small[0:256] = FDo
    small[256:400, 0:128] = FD0
    small[256:384, 128:256] = FD2
    small[400:656] = IDo
    small[656:784, 0:128] = ID0
    small[656:784, 128:256] = ID2
    small[784:912, 0:128] = J2
    tb = np.zeros((288, 128))
    th = 2 * np.pi * np.outer(np.arange(128), np.arange(128)) / 128
    tb[0:128] = np.cos(th); tb[128:256] = -np.sin(th)
    th = 2 * np.pi * np.outer(np.arange(16), np.arange(128)) / S
    tb[256:272] = np.cos(th); tb[272:288] = -np.sin(th)
    return tb.astype(np.float32), small.astype(np.float32)


class _C:
    __slots__ = ("r", "i", "sr", "si")

    def __init__(self, r, i, sr=1, si=1):
        self.r, self.i, self.sr, self.si = r, i, sr, si


def _add(a, sa, b, sb):
    if sa == sb:
        return a + b, sa
    if sa == 1:
        return a - b, 1
    return b - a, 1


def _cadd(a, b):
    r, sr = _add(a.r, a.sr, b.r, b.sr); i, si = _add(a.i, a.si, b.i, b.si)
    return _C(r, i, sr, si)


def _csub(a, b):
    r, sr = _add(a.r, a.sr, b.r, -b.sr); i, si = _add(a.i, a.si, b.i, -b.si)
    return _C(r, i, sr, si)


def _cmul_i(a, s):
    return _C(a.i, a.r, -s * a.si, s * a.sr)


def _ctw(a, num, den, sign):
    num %= den
    if num == 0:
        return a
    if 4 * num == den:
        return _cmul_i(a, sign)
    if 2 * num == den:
        return _C(a.r, a.i, -a.sr, -a.si)
    if 4 * num == 3 * den:
        return _cmul_i(a, -sign)
    th = sign * 2 * np.pi * num / den
    c, s = np.cos(th), np.sin(th)
    if (8 * num) % den == 0:
        h = float(np.sqrt(0.5))
        sc_, ss = int(np.sign(c)), int(np.sign(s))
        r, sr = _add(a.r, sc_ * a.sr, a.i, -ss * a.si)
        i, si = _add(a.r, ss * a.sr, a.i, sc_ * a.si)
        return _C(r * (h * sr), i * (h * si), 1, 1)
    c, s = float(c), float(s)
    return _C(a.r * (a.sr * c) - a.i * (a.si * s), a.r * (a.sr * s) + a.i * (a.si * c), 1, 1)


def _dft4(x, sign):
    a, b, c, d = x
    t0 = _cadd(a, c); t1 = _csub(a, c); t2 = _cadd(b, d); t3 = _cmul_i(_csub(b, d), sign)
    return [_cadd(t0, t2), _cadd(t1, t3), _csub(t0, t2), _csub(t1, t3)]


def _fin(a):
    return (a.r if a.sr == 1 else -a.r), (a.i if a.si == 1 else -a.i)


def _nn(a, b):
    return jax.lax.dot_general(a, b, (((1,), (0,)), ((), ())), preferred_element_type=f32)


def _nt(a, b):
    return jax.lax.dot_general(a, b, (((1,), (1,)), ((), ())), preferred_element_type=f32)


def _tn(a, b):
    return jax.lax.dot_general(a, b, (((0,), (0,)), ((), ())), preferred_element_type=f32)


def _ln_stats(v):
    mu = jnp.mean(v, axis=-1, keepdims=True)
    c = v - mu
    var = jnp.mean(c * c, axis=-1, keepdims=True)
    rstd = jax.lax.rsqrt(var + EPS)
    return c * rstd, rstd


def _ln_bwd(dy, xhat, rstd):
    m1 = jnp.mean(dy, axis=-1, keepdims=True)
    m2 = jnp.mean(dy * xhat, axis=-1, keepdims=True)
    return rstd * (dy - m1 - xhat * m2)


def _perm(v):
    return jnp.swapaxes(v.reshape(16, 16, v.shape[-1]), 0, 1)


class _NS:
    def __init__(self, d):
        self._d = d

    def __getattr__(self, k):
        return self._d[k]


_V = pltpu.VMEM
_INS = ("x_hbm", "wr_hbm", "wi_hbm", "wg_hbm", "wu_hbm", "wd_hbm", "go_hbm", "tb_hbm", "sm_hbm")
_OUTS = ("out_hbm", "dx_hbm", "dwr_hbm", "dwi_hbm", "dwg_hbm", "dwu_hbm", "dwd_hbm")
_SCRATCH = dict(
    x_s=_V((S, D), bf16), go_s=_V((S, D), bf16), wr_s=_V((NM, S), bf16), wi_s=_V((NM, S), bf16),
    wg_s=_V((F, D), bf16), wu_s=_V((F, D), bf16), wd_s=_V((F, D), bf16),
    tb_s=_V((288, 128), f32), sm_s=_V((912, 256), bf16), ms_s=_V((16, 4, 128, 128), bf16),
    xp_s=_V((16, 128, D), bf16), gop_s=_V((16, 128, D), bf16), xh1_s=_V((16, 128, D), bf16), rs1_s=_V((S, 1), f32),
    h_s=_V((S, D), bf16), ln2_s=_V((S, D), bf16), rs_s=_V((S, 1), f32),
    dh_s=_V((S, D), f32), on_s=_V((4, S, 128), f32), dxp_s=_V((16, 128, D), bf16), Tb=_V((16, 128, 640), bf16),
    AT=_V((2, 16, NR, 128), f32), XT=_V((2, 16, NR, 128), f32), WT=_V((2, 16, NR, 128), f32), Y=_V((2, 16, NR, 128), f32),
    Cb=_V((16, 256, 256), bf16), zn_s=_V((2, 16, 8, 128), f32),
    dhh_s=_V((16, 128, F), bf16), dgT_s=_V((F, S), bf16), duT_s=_V((F, S), bf16), hhT_s=_V((F, S), bf16),
    acc_s=_V((2, F, 128), f32),
    out_s=_V((S, D), bf16), dx_s=_V((S, D), bf16), dwr_s=_V((NM, S), bf16), dwi_s=_V((NM, S), bf16),
    dwg_s=_V((F, D), bf16), dwu_s=_V((F, D), bf16), dwd_s=_V((F, D), bf16),
    sem_in=pltpu.SemaphoreType.DMA((10,)), sem_x=pltpu.SemaphoreType.DMA((NT,)), sem_go=pltpu.SemaphoreType.DMA((NT,)),
    sem_out=pltpu.SemaphoreType.DMA((8,)), sem_bar=pltpu.SemaphoreType.REGULAR,
)


def _steps(r):
    AT, XT, WT, Y, Cb, Tb, sm_s, ms_s = r.AT, r.XT, r.WT, r.Y, r.Cb, r.Tb, r.sm_s, r.ms_s

    def FD0(): return sm_s[256:400, 0:128]
    def FD2(): return sm_s[256:384, 128:256]
    def IDo(): return sm_s[400:656, :]
    def ID0(): return sm_s[656:784, 0:128]
    def ID2(): return sm_s[656:784, 128:256]

    def perm_step(dst, src, c, j):
        cols = slice(128 * j, 128 * (j + 1))
        dst[:, 16 * c:16 * (c + 1), cols] = _perm(src[c * TS:(c + 1) * TS, cols])

    def unperm_step(dst, src, c, j):
        cols = slice(128 * j, 128 * (j + 1))
        dst[c * TS:(c + 1) * TS, cols] = jnp.swapaxes(src[:, 16 * c:16 * (c + 1), cols], 0, 1).reshape(TS, 128)

    def cast_step(c, j):
        r.out_s[c * TS:(c + 1) * TS, 128 * j:128 * (j + 1)] = r.on_s[j, c * TS:(c + 1) * TS, :].astype(bf16)

    def gen_ms(s1):
        tb_s = r.tb_s
        fr = tb_s[0:128, :]; fi = tb_s[128:256, :]
        tr = tb_s[256 + s1:257 + s1, :]; ti = tb_s[272 + s1:273 + s1, :]
        mr = fr * tr - fi * ti; mi = fr * ti + fi * tr
        ms_s[s1, 0] = mr.astype(bf16); ms_s[s1, 1] = mi.astype(bf16)
        ms_s[s1, 2] = (mr + mi).astype(bf16); ms_s[s1, 3] = (mr - mi).astype(bf16)

    def wprep(p, a):
        w_s = (r.wr_s, r.wi_s)[p]
        cols = slice(128 * a, 128 * (a + 1))
        u = pltpu.bitcast(w_s[0:256, cols], jnp.uint32)
        ev = pltpu.bitcast(u << 16, f32); od = pltpu.bitcast(u & jnp.uint32(0xFFFF0000), f32)
        u2 = pltpu.bitcast(ev.astype(bf16), jnp.uint32)
        WT[p, a, 0:64, :] = pltpu.bitcast(u2 << 16, f32)
        WT[p, a, 64:128, :] = pltpu.bitcast(u2 & jnp.uint32(0xFFFF0000), f32)
        WT[p, a, 128:256, :] = od
        WT[p, a, 256:264, :] = jnp.broadcast_to(w_s[256:257, cols].astype(f32), (8, 128))

    def wsym(row, p):
        lane0 = jax.lax.broadcasted_iota(jnp.int32, (1, 128), 1) == 0
        R = jnp.concatenate([WT[p, a, row:row + 1, :] for a in range(16)], axis=0)
        A2 = _nn(R.astype(bf16), sm_s[784:912, 0:128])
        sg = 0.5 if p == 0 else -0.5
        for a in range(16):
            rev = jnp.where(lane0, A2[(16 - a) % 16:(16 - a) % 16 + 1], A2[15 - a:16 - a])
            WT[p, a, row:row + 1, :] = 0.5 * R[a:a + 1] + sg * rev

    def dwpost(p, a):
        dw_s = (r.dwr_s, r.dwi_s)[p]
        cols = slice(128 * a, 128 * (a + 1))

        def bits(x):
            return pltpu.bitcast(x.astype(bf16).astype(f32), jnp.uint32)

        evb = pltpu.bitcast((bits(AT[p, a, 0:64, :]) >> 16) | bits(AT[p, a, 64:128, :]), bf16)
        w = (pltpu.bitcast(evb.astype(f32), jnp.uint32) >> 16) | bits(AT[p, a, 128:256, :])
        dw_s[0:256, cols] = pltpu.bitcast(w, bf16)
        dw_s[256:257, cols] = AT[p, a, 256:257, :].astype(bf16)

    def radix4(L):
        l0, l1, l2, l3 = (L[:, 128 * j:128 * (j + 1)] for j in range(4))
        e = l0 + l2; o = l1 + l3
        p = l0 - l2; q = l1 - l3
        return jnp.concatenate([e + o, e - o, p, q, p + q], axis=1).astype(bf16)

    def fwd_mm(q, s1):
        o0 = _nt(FD0(), q[:, 0:128]); o2 = _nt(FD2(), q[:, 128:256])
        k1 = _nt(sm_s[0:128, 0:128], q[:, 512:640])
        k2 = _nt(sm_s[0:128, 128:256], q[:, 256:384]); k3 = _nt(sm_s[128:256, 0:128], q[:, 384:512])
        even = (jax.lax.broadcasted_iota(jnp.int32, (128, 128), 0) & 1) == 0
        Ar = jnp.concatenate([o0[0:64], o2[0:64], k1 + k3, o0[64:80]], axis=0)
        Ai = jnp.concatenate([o0[80:144], o2[64:128], k2 + jnp.where(even, -k1, k1)], axis=0)
        As = jnp.concatenate([Ar[0:256] + Ai, Ar[256:272]], axis=0).astype(bf16)
        Ar = Ar.astype(bf16)
        Ai = jnp.concatenate([Ai.astype(bf16), jnp.zeros((16, 128), bf16)], axis=0)
        t1 = _nn(Ar, ms_s[s1, 0]); t2 = _nn(Ai, ms_s[s1, 1]); t3 = _nn(As, ms_s[s1, 2])
        AT[0, s1] = t1 - t2
        AT[1, s1] = t3 - (t1 + t2)

    def c_mm(s1):
        fwd_mm(Tb[s1], s1)

    def p1(s1):
        L, rstd = _ln_stats(r.xp_s[s1].astype(f32))
        r.xh1_s[s1] = L.astype(bf16)
        r.rs1_s[s1 * 128:(s1 + 1) * 128, :] = rstd
        fwd_mm(radix4(L), s1)

    def sp_alpha(g, n2):
        rows = slice(8 * g, 8 * g + 8)
        y = _dft4([_C(AT[0, 4 * n1 + n2, rows, :], AT[1, 4 * n1 + n2, rows, :]) for n1 in range(4)], -1)
        for k1 in range(4):
            re, im = _fin(_ctw(y[k1], k1 * n2, 16, -1))
            Y[0, 4 * k1 + n2, rows, :] = re; Y[1, 4 * k1 + n2, rows, :] = im

    def sp_beta(g, k1, bwd):
        rows = slice(8 * g, 8 * g + 8)
        row0 = jax.lax.broadcasted_iota(jnp.int32, (8, 128), 0) == 0
        o = _dft4([_C(Y[0, 4 * k1 + n2, rows, :], Y[1, 4 * k1 + n2, rows, :]) for n2 in range(4)], -1)
        Z = []
        for k2 in range(4):
            k = k1 + 4 * k2
            ar, ai = _fin(o[k2])
            wr = WT[0, k, rows, :]; wi = WT[1, k, rows, :]
            if not bwd:
                XT[0, k, rows, :] = ar; XT[1, k, rows, :] = ai
                zr = ar * wr - ai * wi; zi = ar * wi + ai * wr
            else:
                xr = XT[0, k, rows, :]; xi = XT[1, k, rows, :]
                if g in (0, 32):
                    cm = jnp.where(row0, 1.0 / (S * D), 2.0 / (S * D)).astype(f32)
                else:
                    cm = 2.0 / (S * D)
                AT[0, k, rows, :] = (ar * xr + ai * xi) * cm
                AT[1, k, rows, :] = (ai * xr - ar * xi) * cm
                zr = ar * wr + ai * wi; zi = ai * wr - ar * wi
            if g == 32:
                r.zn_s[0, k] = zr; r.zn_s[1, k] = zi
            else:
                if g == 0:
                    zr = zr - jnp.where(row0, r.zn_s[1, k, 0:1, :], 0.0)
                    zi = zi + jnp.where(row0, r.zn_s[0, k, 0:1, :], 0.0)
                Z.append(_C(zr, zi))
        if g != 32:
            v = _dft4(Z, +1)
            for sb in range(4):
                re, im = _fin(_ctw(v[sb], k1 * sb, 16, +1))
                Y[0, 4 * k1 + sb, rows, :] = re; Y[1, 4 * k1 + sb, rows, :] = im

    def sp_gamma(g, sb):
        rows = slice(8 * g, 8 * g + 8)
        o = _dft4([_C(Y[0, 4 * k1 + sb, rows, :], Y[1, 4 * k1 + sb, rows, :]) for k1 in range(4)], +1)
        for sa in range(4):
            re, im = _fin(o[sa])
            Cb[4 * sa + sb, rows, 0:128] = re.astype(bf16); Cb[4 * sa + sb, rows, 128:256] = im.astype(bf16)

    def spectral_steps(bwd):
        st = []
        for g in [32] + list(range(32)):
            st += [(30, P(sp_alpha, g, q)) for q in range(4)]
            st += [(70 if g != 32 else 50, P(sp_beta, g, q, bwd)) for q in range(4)]
            if g != 32:
                st += [(30, P(sp_gamma, g, q)) for q in range(4)]
        return st

    def inv1(s1):
        lane_lo = jax.lax.broadcasted_iota(jnp.int32, (128, 128), 1) < 64
        C = Cb[s1]
        cr = C[:, 0:128]; ci = C[:, 128:256]
        cs = (cr.astype(f32) + ci.astype(f32)).astype(bf16)
        t1 = _nt(ms_s[s1, 0], cr); t2 = _nt(ms_s[s1, 1], ci); t3 = _nt(ms_s[s1, 3], cs)
        Tr = t1 + t2
        Ti = t3 + (t2 - t1)
        tr0 = Tr[:, 0:128]; ti0 = Ti[:, 0:128]
        Tb[s1, :, 0:128] = jnp.where(lane_lo, tr0, pltpu.roll(ti0, 64, 1)).astype(bf16)
        Tb[s1, :, 128:256] = jnp.where(lane_lo, pltpu.roll(tr0, 64, 1), ti0).astype(bf16)
        Tb[s1, :, 256:384] = Tr[:, 128:256].astype(bf16)
        Tb[s1, :, 384:512] = Ti[:, 128:256].astype(bf16)

    def inv2(b0, nb):
        tb = Tb[b0:b0 + nb, :, 0:512].reshape(nb * 128, D)
        U0 = _nn(tb[:, 0:128], ID0()); U2 = _nn(tb[:, 128:256], ID2()); Uo = _nn(tb[:, 256:512], IDo())
        a = U0 + U2; b = U0 - U2
        U1a = Uo[:, 0:128]; U1b = Uo[:, 128:256]
        return jnp.concatenate([a + U1a, b + U1b, a - U1a, b - U1b], axis=1)

    def a2(b0, nb):
        rows = slice(b0 * 128, (b0 + nb) * 128)
        h = r.xp_s[b0:b0 + nb].reshape(nb * 128, D).astype(f32) + inv2(b0, nb)
        xh2, rstd2 = _ln_stats(h)
        r.h_s[rows, :] = h.astype(bf16)
        r.ln2_s[rows, :] = xh2.astype(bf16)
        r.rs_s[rows, :] = rstd2

    def p52(b0, nb):
        rows = slice(b0 * 128, (b0 + nb) * 128)
        dL = inv2(b0, nb)
        res = r.dh_s[rows, :] + _ln_bwd(dL, r.xh1_s[b0:b0 + nb].reshape(nb * 128, D).astype(f32), r.rs1_s[rows, :])
        r.dxp_s[b0:b0 + nb] = res.astype(bf16).reshape(nb, 128, D)

    def dhh_piece(s1, n, a=0, b=128):
        n0 = 128 * n; n1 = min(F, n0 + 128)
        r.dhh_s[s1, a:b, n0:n1] = _nt(r.gop_s[s1, a:b, :], r.wd_s[n0:n1, :]).astype(bf16)

    def dhh_cpiece(c, n):
        n0 = 128 * n; n1 = min(F, n0 + 128)
        g = r.gop_s[:, 16 * c:16 * (c + 1), :].reshape(TS, D)
        r.dhh_s[:, 16 * c:16 * (c + 1), n0:n1] = _nt(g, r.wd_s[n0:n1, :]).astype(bf16).reshape(16, 16, n1 - n0)

    def b_stage(t, c):
        rows = pl.ds(pl.multiple_of(t * TS, TS), TS)
        blk = pl.ds(2 * t, 2)
        ln2 = r.ln2_s[rows, :]
        ln2T = ln2.T
        gT = _nn(r.wg_s[...], ln2T); uT = _nn(r.wu_s[...], ln2T)
        hhT = (gT * uT).astype(bf16)
        r.hhT_s[:, rows] = hhT
        dhhT = r.dhh_s[blk].reshape(TS, F).T.astype(f32)
        dgT = (dhhT * uT).astype(bf16); duT = (dhhT * gT).astype(bf16)
        r.dgT_s[:, rows] = dgT; r.duT_s[:, rows] = duT
        dl = _tn(dgT, r.wg_s[...]) + _tn(duT, r.wu_s[...])
        dh = r.gop_s[blk].reshape(TS, D).astype(f32) + _ln_bwd(dl, ln2.astype(f32), r.rs_s[rows, :])
        r.dh_s[rows, :] = dh
        Tb[blk] = radix4(dh).reshape(2, 128, 640)
        o = r.h_s[rows, :].astype(f32) + _tn(hhT, r.wd_s[...])
        for hf in range(2):
            for j in range(4):
                r.on_s[j, pl.ds(2 * t + hf, 128, stride=16), :] = o[128 * hf:128 * (hf + 1), 128 * j:128 * (j + 1)]
        return c

    def _dw_refs(mat):
        return (r.hhT_s, r.dgT_s, r.duT_s)[mat], (r.dwd_s, r.dwg_s, r.dwu_s)[mat]

    def dwk_piece(mat, n, kc, r0, r1, KC=512):
        lhs, dst = _dw_refs(mat)
        nb = KC // 128
        if mat == 0:
            rhs = r.gop_s[nb * kc:nb * (kc + 1), :, 128 * n:128 * (n + 1)].reshape(KC, 128)
        else:
            rhs = r.ln2_s[KC * kc:KC * (kc + 1), 128 * n:128 * (n + 1)]
        res = _nn(lhs[r0:r1, KC * kc:KC * (kc + 1)], rhs)
        acc = r.acc_s.at[n % 2]
        if kc == 0:
            acc[r0:r1, :] = res
        elif kc < S // KC - 1:
            acc[r0:r1, :] = acc[r0:r1, :] + res
        else:
            dst[r0:r1, 128 * n:128 * (n + 1)] = (acc[r0:r1, :] + res).astype(bf16)

    def dwk_col(mat, n, rows):
        mp = [(a, min(F, a + rows)) for a in range(0, F, rows)]
        return [P(dwk_piece, mat, n, kc, a, b) for kc in range(S // 512) for (a, b) in mp]

    def dw_col(mat, n):
        lhs, dst = _dw_refs(mat)
        cols = slice(128 * n, 128 * (n + 1)) if isinstance(n, int) else pl.ds(pl.multiple_of(n * 128, 128), 128)
        rhs = r.gop_s[:, :, cols].reshape(S, 128) if mat == 0 else r.ln2_s[:, cols]
        dst[:, cols] = _nn(lhs[...], rhs).astype(bf16)

    def barrier():
        pl.semaphore_signal(r.sem_bar, 1)
        pl.semaphore_wait(r.sem_bar, 1)

    return _NS(dict(
        perm_step=perm_step, cast_step=cast_step, unperm_step=unperm_step, gen_ms=gen_ms, wprep=wprep, wsym=wsym, dwpost=dwpost,
        p1=p1, c_mm=c_mm, spectral_steps=spectral_steps, inv1=inv1, a2=a2, p52=p52,
        dhh_piece=dhh_piece, dhh_cpiece=dhh_cpiece, b_stage=b_stage, dwk_col=dwk_col, dw_col=dw_col, barrier=barrier))


def _weave(chain, fill):
    tot = sum(w for w, _ in chain)
    acc = 0.0; done = 0
    for w, fn in chain:
        fn(); acc += w
        upto = int(round(len(fill) * acc / tot))
        for f in fill[done:upto]:
            f()
        done = upto
    for f in fill[done:]:
        f()


def _schedule(r, w):
    sc = jax.named_scope
    cp = pltpu.make_async_copy
    cx = [cp(r.x_hbm.at[pl.ds(c * TS, TS)], r.x_s.at[pl.ds(c * TS, TS)], r.sem_x.at[c]) for c in range(NT)]
    cgo = [cp(r.go_hbm.at[pl.ds(c * TS, TS)], r.go_s.at[pl.ds(c * TS, TS)], r.sem_go.at[c]) for c in range(NT)]

    def rows_cp(src, dst, a, n, i):
        return cp(src.at[pl.ds(a, n)], dst.at[pl.ds(a, n)], r.sem_in.at[i])

    cwd = [rows_cp(r.wd_hbm, r.wd_s, 0, 512, 0), rows_cp(r.wd_hbm, r.wd_s, 512, F - 512, 1)]
    csm = [rows_cp(r.sm_hbm, r.sm_s, 0, 400, 2), rows_cp(r.sm_hbm, r.sm_s, 400, 512, 3)]
    ctb = cp(r.tb_hbm, r.tb_s, r.sem_in.at[4])
    cwr = cp(r.wr_hbm, r.wr_s, r.sem_in.at[5]); cwi = cp(r.wi_hbm, r.wi_s, r.sem_in.at[6])
    cwg = cp(r.wg_hbm, r.wg_s, r.sem_in.at[7]); cwu = cp(r.wu_hbm, r.wu_s, r.sem_in.at[8])

    def perms(cs):
        return [(1, P(w.perm_step, r.gop_s, r.go_s, c, j)) for c in cs for j in range(4)]

    def cps(cs):
        return [P(w.dhh_cpiece, c, n) for c in cs for n in range(4)]

    with sc("h0"):
        ctb.start(); cwd[0].start(); cgo[0].start()
        ctb.wait()
        for s1 in range(16):
            w.gen_ms(s1)
    with sc("h1"):
        cwd[0].wait(); cgo[0].wait()
        for c in cgo[1:]: c.start()
        csm[0].start()
        for c in cx: c.start()
        for _, f in perms([0]): f()
        for f in cps([0]): f()
    with sc("h2"):
        cgo[1].wait(); cgo[2].wait()
        for _, f in perms([1]): f()
        _weave(perms([2]), cps([1]))
        for f in cps([2]): f()
    with sc("h2b"):
        cgo[3].wait(); cgo[4].wait(); cgo[5].wait()
        for _, f in perms([3]): f()
        _weave(perms([4, 5]), cps([3]))
        for f in cps([4, 5]): f()
    with sc("h3"):
        cgo[6].wait(); cgo[7].wait()
        for c in range(4):
            cx[c].wait()
        xp = [(1, P(w.perm_step, r.xp_s, r.x_s, c, j)) for c in range(4) for j in range(4)]
        for _, f in perms([6]): f()
        _weave(perms([7]) + xp[0:8], cps([6]))
        _weave(xp[8:16], cps([7]))
    H = [P(w.dhh_piece, s1, n) for n in range(4, 11) for s1 in range(16)]
    with sc("h5_xperm"):
        for c in range(4, NT):
            cx[c].wait()
        csm[0].wait()
        cwd[1].start(); csm[1].start(); cwr.start(); cwi.start()
        for c in range(4, NT):
            for j in range(4):
                w.perm_step(r.xp_s, r.x_s, c, j)
    with sc("h6_p1"):
        for s1 in range(16):
            w.p1(s1)
    with sc("h7_wprep"):
        cwd[1].wait(); csm[1].wait(); cwr.wait(); cwi.wait()
        w.barrier()
        _weave([(1, P(w.wprep, p, a)) for a in range(16) for p in range(2)]
               + [(1, P(w.wsym, row, p)) for row in (0, 256) for p in range(2)], H[0:16])
        w.barrier()
    with sc("h8_spec"):
        cwg.start(); cwu.start()
        _weave(w.spectral_steps(False), [P(f, a, a + 64) for f in H[16:80] for a in (0, 64)])
        w.barrier()
    with sc("h9_a"):
        for s1 in range(16):
            w.inv1(s1)
        _weave([(1, P(w.a2, s1, 1)) for s1 in range(16)], H[80:112])

    with sc("b_loop"):
        cwg.wait(); cwu.wait()
        jax.lax.fori_loop(0, NT, w.b_stage, 0)

    outs = []

    def out_dma(src, dst, i):
        c = cp(src, dst, r.sem_out.at[i]); c.start(); outs.append(c)

    def col(a, b, rows):
        return [f for q in range(a, b) for f in w.dwk_col(q // 4, q % 4, rows)]

    def unp(dst, src):
        return [(1, P(w.unperm_step, dst, src, c, j)) for c in range(NT) for j in range(4)]

    with sc("w2_c"):
        for s1 in range(16):
            w.c_mm(s1)
        w.barrier()
    with sc("w3_spec"):
        _weave(w.spectral_steps(True), col(0, 5, 96))
        w.barrier()
    with sc("w4_p5"):
        out_dma(r.dwd_s, r.dwd_hbm, 3)
        for s1 in range(16):
            w.inv1(s1)
        _weave([(1, P(w.p52, s1, 1)) for s1 in range(16)], col(5, 6, 256))
        w.barrier()
    with sc("w5_post"):
        _weave([(1, P(w.cast_step, c, j)) for c in range(NT) for j in range(4)] + [(1, P(w.dwpost, p, a)) for a in range(16) for p in range(2)]
               + unp(r.dx_s, r.dxp_s), col(6, 8, 128))
        w.barrier()
    with sc("w7_loop"):
        out_dma(r.out_s, r.out_hbm, 0); out_dma(r.dx_s, r.dx_hbm, 6)
        out_dma(r.dwr_s, r.dwr_hbm, 4); out_dma(r.dwi_s, r.dwi_hbm, 5); out_dma(r.dwg_s, r.dwg_hbm, 1)

        c3 = cp(r.dwu_s.at[:, 0:384], r.dwu_hbm.at[:, 0:384], r.sem_out.at[2])

        def colbody(n, c):
            @pl.when(n == 3)
            def _():
                c3.start()
            w.dw_col(2, n)
            return c
        jax.lax.fori_loop(0, 4, colbody, 0)
        outs.append(c3)
    with sc("w9_tail"):
        c4 = cp(r.dwu_s.at[:, 384:512], r.dwu_hbm.at[:, 384:512], r.sem_out.at[7]); c4.start(); outs.append(c4)
        for c in outs:
            c.wait()


def _build(schedule):
    names = _INS + _OUTS + tuple(_SCRATCH)

    def kernel(*refs):
        r = _NS(dict(zip(names, refs)))
        schedule(r, _steps(r))

    def run(A_x, A_w_r, A_w_i, B_w_gate, B_w_up, B_w_down, grad_out):
        tbl, small = _consts()
        tb = jnp.asarray(tbl, f32); sm = jnp.asarray(small, bf16)
        any_spec = pl.BlockSpec(memory_space=pl.ANY)
        sds = jax.ShapeDtypeStruct
        outs = pl.pallas_call(
            kernel,
            out_shape=(sds((S, D), bf16), sds((S, D), bf16), sds((NM, S), bf16), sds((NM, S), bf16),
                       sds((F, D), bf16), sds((F, D), bf16), sds((F, D), bf16)),
            in_specs=[any_spec] * len(_INS),
            out_specs=tuple([any_spec] * len(_OUTS)),
            scratch_shapes=list(_SCRATCH.values()),
            compiler_params=pltpu.CompilerParams(vmem_limit_bytes=110 * 1024 * 1024),
        )(A_x.reshape(S, D), A_w_r.T, A_w_i.T, B_w_gate.T, B_w_up.T, B_w_down, grad_out.reshape(S, D), tb, sm)
        out, dx, dwrT, dwiT, dwgT, dwuT, dwd = outs
        return (out.reshape(1, S, D), dx.reshape(1, S, D), dwrT.T, dwiT.T, dwgT.T, dwuT.T, dwd)

    return run


@jax.jit
def pallas_sequential_preLN__spectral_gfnet__glu_gated_bilinear__prompt_kernel(
        A_x, A_w_r, A_w_i, B_x, B_w_gate, B_w_up, B_w_down, grad_out):
    del B_x
    return _build(_schedule)(A_x, A_w_r, A_w_i, B_w_gate, B_w_up, B_w_down, grad_out)
```
